```python
import os as _os
_os.environ.setdefault("JAX_PLATFORMS", "cpu")
import jax
import jax.numpy as jnp

def _softmax(x, axis=-1):
    return jax.nn.softmax(x, axis=axis)
def _gelu(x):
    return jax.nn.gelu(x, approximate=True)
def _silu(x):
    return jax.nn.silu(x)
def _sigmoid(x):
    return jax.nn.sigmoid(x)
def _layernorm(x, axis=-1, eps=1e-5):
    m = jnp.mean(x, axis=axis, keepdims=True)
    v = jnp.var(x, axis=axis, keepdims=True)
    return (x - m) / jnp.sqrt(v + eps)
def _scatter_add(tgt, idx, src, axis=0):
    return tgt.at[idx].add(src)
def _segment_sum(src, seg, n):
    return jax.ops.segment_sum(src, seg, n)
class _Rng:
    def __init__(self, key):
        self._k = key
    def _next(self):
        self._k, sub = jax.random.split(self._k)
        return sub
    def normal(self, shape):
        return jax.random.normal(self._next(), shape, dtype=jnp.bfloat16)
    def randint(self, lo, hi, shape):
        return jax.random.randint(self._next(), shape, lo, hi, dtype=jnp.int32)
    def uniform(self, shape, lo=0.0, hi=1.0):
        return jax.random.uniform(self._next(), shape, jnp.bfloat16, lo, hi)
    def permutation(self, n):
        return jax.random.permutation(self._next(), n)


kernel_name = 'standalone__batchnorm__sampling'

def setup_inputs():
    _rng = _Rng(jax.random.key(int.from_bytes(__import__("os").urandom(4), "little")))
    _w = (lambda a: (lambda t: t.astype(jnp.bfloat16) if jnp.issubdtype(t.dtype, jnp.floating) else t)(jnp.asarray(a)))
    B, S, C = 1024, 8, 640
    K = 3
    return {
        "x": _w((lambda *s: _rng.normal(s) * 0.05)(B, S, C)),
        "w": _w((lambda *s: _rng.normal(s) * 0.05)(K, C, C) * (1.0 / (K * C) ** 0.5)),
        "mean": _w((lambda *s: _rng.normal(s) * 0.05)(C) * 0.1),
        "var": _w(jnp.abs((lambda *s: _rng.normal(s) * 0.05)(C)) + 0.5),
        "g": _w((lambda *s: _rng.normal(s) * 0.05)(C) + 1.0),
        "b": _w((lambda *s: _rng.normal(s) * 0.05)(C) * 0.1),
    }

def reference(x, w, mean, var, g, b):
    K = 3
    P = K // 2
    S = x.shape[1]
    xp = jnp.pad(x, ((0, 0), (P, P), (0, 0)))
    y = sum(jnp.einsum('bsc,cd->bsd', xp[:, k:k + S, :], w[k]) for k in range(K))
    inv_std = 1.0 / jnp.sqrt(var + 1e-5)
    y = (y - mean) * (g * inv_std) + b
    return _silu(y)
```

```python
import jax
import jax.numpy as jnp
from jax import lax
import jax.experimental.pallas as pl
import jax.experimental.pallas.tpu as pltpu

A = 1.6
A2 = A * A
KAP = 1.0 / (A ** 4 - 1.0)
LAM = KAP / 2
K2 = (A ** 4 + 1) / A2
f32 = jnp.float32
u32 = jnp.uint32
bf16 = jnp.bfloat16

TB = 64
TG = 16
XPRE = 5
NPK = 40
TGATE = ((0, 120), (1, 120), (2, 120), (3, 120))
JORD = (1, 2, 3, 4, 0, 5)
WG = ((None, 0), (0, 0), (0, 120), (1, 0))
SG = ((4, 120), (5, 120), (6, 120), (7, 120))


@jax.jit
def pallas_standalone__batchnorm__sampling_kernel(
    x: jax.Array,
    w: jax.Array,
    mean: jax.Array,
    var: jax.Array,
    g: jax.Array,
    b: jax.Array,
):
    B, S, C = x.shape
    assert S == 8 and w.shape[0] == 3
    x2 = x.reshape(B * S, C)
    TM = TB * S
    R = 2 * TB
    NB = C // 128
    NC = B // TB
    NQ = TB // TG

    def kernel(x_hbm, w_hbm, mean_hbm, var_hbm, g_hbm, b_hbm, o_hbm,
               xbuf, obuf, wbuf, v_ref, ua_ref, ub_ref, uc_ref, pb0, pb1, pb2, pb3,
               p_ref, pk_ref, sx, so, sw, sp):
        pbuf = (pb0, pb1, pb2, pb3)

        def xcopy(i, k):
            return pltpu.make_async_copy(
                x_hbm.at[pl.ds(i * TM, TM), pl.ds(k * 128, 128)],
                xbuf.at[i, k].bitcast(bf16), sx.at[i])

        def ocopy(i, k):
            return pltpu.make_async_copy(
                obuf.at[i, k].bitcast(bf16),
                o_hbm.at[pl.ds(i * TM, TM), pl.ds(k * 128, 128)], so.at[i])

        def wcopy(t, n):
            return pltpu.make_async_copy(
                w_hbm.at[t, :, pl.ds(pl.multiple_of(n * 128, 128), 128)],
                wbuf.at[t, n].bitcast(bf16), sw.at[n])

        pcopies = [pltpu.make_async_copy(h, pbuf[q], sp.at[0])
                   for q, h in enumerate((mean_hbm, var_hbm, g_hbm, b_hbm))]

        def issue_x(i, c):
            for k in range(NB):
                xcopy(i, k).start()
            return c

        def issue_w(n, c):
            for t in range(3):
                wcopy(t, n).start()
            return c

        lax.fori_loop(0, 2, issue_x, 0)
        for c in pcopies:
            c.start()
        lax.fori_loop(0, NB, issue_w, 0)
        lax.fori_loop(2, 2 + XPRE, issue_x, 0)

        def zero_from(m):
            return (lax.bitcast_convert_type(m, u32) >> 16) >> 16

        def gate_f32(c, z):
            if z is None:
                return c
            cb = lax.bitcast_convert_type(jnp.full((8, 128), c, f32), u32)
            return lax.bitcast_convert_type(cb + z, f32)

        def rep(v, rows):
            return v if jnp.ndim(v) == 0 else jnp.concatenate([v] * (rows // 8), axis=0)

        def split(lst, pi, npc):
            return lst[pi * len(lst) // npc:(pi + 1) * len(lst) // npc]

        def transform(i, u_ref, pieces, z=None):
            if z is None:
                shl = jnp.uint32(16)
                msk = jnp.uint32(0xFFFF0000)
            else:
                shl = rep(z + jnp.uint32(16), TG)
                msk = rep(z + jnp.uint32(0xFFFF0000), TG)
            lo_f32 = lambda w_: lax.bitcast_convert_type(w_ << shl, f32)
            hi_f32 = lambda w_: lax.bitcast_convert_type(w_ & msk, f32)
            for (k, t, q) in pieces:
                cs = slice(k * 128, (k + 1) * 128)
                ev = xbuf[i, k, pl.ds(4 * q * TG + 2 * t, TG, stride=4), :]
                od = xbuf[i, k, pl.ds(4 * q * TG + 2 * t + 1, TG, stride=4), :]
                d0 = lo_f32(ev); d1 = hi_f32(ev); d2 = lo_f32(od); d3 = hi_f32(od)
                e1 = d0 + A2 * d2
                o1 = A * d1 + (A * A2) * d3
                e2 = d3 + A2 * d1
                o2 = A * d2 + (A * A2) * d0
                if isinstance(t, int):
                    rr = slice((t * TB + q * TG) // 2, (t * TB + (q + 1) * TG) // 2)
                else:
                    rr = pl.ds(pl.multiple_of(t * (TB // 2) + q * (TG // 2), 8), TG // 2)
                for j, val in enumerate((d0, e1 + o1, e1 - o1, e2 + o2, e2 - o2, d3)):
                    u_ref.at[j][rr, cs] = pltpu.bitcast(val.astype(bf16), u32)

        def wtransform(n, rows, z=None):
            c1 = rep(gate_f32(LAM * A, z), 32)
            c2 = rep(gate_f32(LAM, z), 32)
            c3 = rep(gate_f32(LAM * A2, z), 32)
            for r in rows:
                rp = slice(r * 16, (r + 1) * 16)
                ld = lambda t: pltpu.bitcast(wbuf[t, n, rp, :], bf16).astype(f32)
                h0 = ld(2); h1 = ld(1); h2 = ld(0)
                ho = h1 * c1
                he = h0 * c2 + h2 * c3
                hr = h2 * c2 + h0 * c3
                for j, val in enumerate((he + ho, he - ho, hr + ho, hr - ho)):
                    v_ref.at[j, n][rp, :] = pltpu.bitcast(val.astype(bf16), u32)

        def dotj(u_ref, j, n):
            if j == 0:
                v = wbuf[2, n]
            elif j == 5:
                v = wbuf[0, n]
            else:
                v = v_ref[j - 1, n]
            return jnp.dot(pltpu.bitcast(u_ref[j], bf16), pltpu.bitcast(v, bf16),
                           preferred_element_type=f32)

        slot = [0]

        def epi(i, n, Ms):
            scn = rep(p_ref[0, n], TB)
            shn = rep(p_ref[1, n], TB)

            def act(y):
                h = y * scn + shn
                return h + h * jnp.tanh(h)

            for t in range(2):
                a0, Pp, Pm, Qp, Qm, a5 = [Ms[j][t * TB:(t + 1) * TB] for j in range(6)]
                SP = Pp + Pm; DP = Pp - Pm; SQ = Qp + Qm; DQ = Qp - Qm
                b0 = a0 + Ms[0][TB:] if t == 0 else a0
                b5 = a5 + Ms[5][:TB] if t == 1 else a5
                c4 = (SP + b0) - DQ * (1.0 / A)
                c2 = A * DQ - (SP * (1.0 / A2) + a0 * K2)
                c1 = (SQ - DP * (1.0 / A)) + b5
                c3 = (A * DP - SQ * (1.0 / A2)) - a5 * K2
                for pp, (lo, hi) in enumerate(((c1, c2), (c3, c4))):
                    sl = slot[0]
                    slot[0] = (slot[0] + 2) % NPK
                    pk_ref.at[sl][...] = pltpu.bitcast(act(lo).astype(bf16), u32)
                    pk_ref.at[sl + 1][...] = pltpu.bitcast(act(hi).astype(bf16), u32)
                    P = pk_ref[sl]
                    Q = pk_ref[sl + 1]
                    obuf[i, n, pl.ds(2 * t + pp, TB // 2, stride=8), :] = (
                        (P & jnp.uint32(0xFFFF)) | (Q << 16))
                    obuf[i, n, pl.ds(4 + 2 * t + pp, TB // 2, stride=8), :] = (
                        (P >> 16) | (Q & jnp.uint32(0xFFFF0000)))
            ocopy(i, n).start()

        allp = [(k, t, q) for k in range(NB) for t in range(2) for q in range(NQ)]
        for k in range(NB):
            xcopy(0, k).wait()
        transform(0, uc_ref, allp)
        for k in range(NB):
            xcopy(1, k).wait()
        transform(1, ub_ref, allp)
        for c in pcopies:
            c.wait()
        inv = lax.rsqrt(pbuf[1][...].astype(f32) + 1e-5)
        sc = pbuf[2][...].astype(f32) * inv * 0.5
        sh = pbuf[3][...].astype(f32) * 0.5 - pbuf[0][...].astype(f32) * sc
        sc = sc.reshape(NB, 128)
        sh = sh.reshape(NB, 128)
        for n in range(NB):
            p_ref[0, n] = jnp.broadcast_to(sc[n:n + 1], (8, 128))
            p_ref[1, n] = jnp.broadcast_to(sh[n:n + 1], (8, 128))

        NR = C // 32

        def startup(n, carry):
            for t in range(3):
                wcopy(t, n).wait()

            @pl.when(n == 3)
            def _():
                for k in range(NB):
                    xcopy(2, k).wait()

            src = jnp.where(n >= 3, 2, 0)
            tsel = n & 1
            tp = [(k, tsel, q) for k in range(NB) for q in range(NQ)]
            order = [(0, 0), (0, 5), (1, 0), (1, 5), (0, 1), (0, 2), (0, 3), (0, 4),
                     (1, 1), (1, 2), (1, 3), (1, 4)]
            for gi, (gp, gr) in enumerate(WG):
                if gp is None:
                    wtransform(n, split(list(range(NR)), gi, len(WG)))
            Ms = ({}, {})
            for pos, (c, j) in enumerate(order):
                Ms[c][j] = dotj((uc_ref, ub_ref)[c], j, n)
                for gi, (gp, gr) in enumerate(WG):
                    if gp == pos:
                        wtransform(n, split(list(range(NR)), gi, len(WG)),
                                   zero_from(Ms[c][j][gr:gr + 8]))
                for gi, (gp, gr) in enumerate(SG):
                    if gp == pos:
                        transform(src, ua_ref, split(tp, gi, len(SG)),
                                  zero_from(Ms[c][j][gr:gr + 8]))
                if len(Ms[c]) == 6:
                    epi(c, n, Ms[c])
            return carry

        lax.fori_loop(0, NB, startup, 0)

        NG = (NC - 2) // 2

        def group(gi, carry):
            a = 2 + 2 * gi
            for k in range(NB):
                xcopy(a + 1, k).wait()

            @pl.when(a + 2 < NC)
            def _():
                for k in range(NB):
                    xcopy(a + 2, k).wait()

            for u in range(2):
                i = a + u
                inext = jnp.minimum(i + 1, NC - 1)
                ucur, unext = (ua_ref, ub_ref) if u == 0 else (ub_ref, ua_ref)
                for n in range(NB):
                    tp = [(n, t, q) for t in range(2) for q in range(NQ)]
                    Ms = {}
                    for pos, j in enumerate(JORD):
                        Ms[j] = dotj(ucur, j, n)
                        for gi_, (gp, gr) in enumerate(TGATE):
                            if gp == pos:
                                transform(inext, unext, split(tp, gi_, len(TGATE)),
                                          zero_from(Ms[j][gr:gr + 8]))
                    epi(i, n, Ms)
            for d in range(2):
                @pl.when(a + XPRE + d < NC)
                def _():
                    for k in range(NB):
                        xcopy(a + XPRE + d, k).start()
            return carry

        lax.fori_loop(0, NG, group, 0)
        for i in range(NC):
            for k in range(NB):
                ocopy(i, k).wait()

    anyspec = pl.BlockSpec(memory_space=pl.ANY)
    out = pl.pallas_call(
        kernel,
        in_specs=[anyspec] * 6,
        out_specs=anyspec,
        out_shape=jax.ShapeDtypeStruct((B * S, C), x.dtype),
        scratch_shapes=[
            pltpu.VMEM((NC, NB, TM // 2, 128), u32),
            pltpu.VMEM((NC, NB, TM // 2, 128), u32),
            pltpu.VMEM((3, NB, C // 2, 128), u32),
            pltpu.VMEM((4, NB, C // 2, 128), u32),
            pltpu.VMEM((6, R // 2, C), u32),
            pltpu.VMEM((6, R // 2, C), u32),
            pltpu.VMEM((6, R // 2, C), u32),
            pltpu.VMEM((C,), bf16), pltpu.VMEM((C,), bf16),
            pltpu.VMEM((C,), bf16), pltpu.VMEM((C,), bf16),
            pltpu.VMEM((2, NB, 8, 128), f32),
            pltpu.VMEM((NPK, TB // 2, 128), u32),
            pltpu.SemaphoreType.DMA((NC,)), pltpu.SemaphoreType.DMA((NC,)),
            pltpu.SemaphoreType.DMA((NB,)), pltpu.SemaphoreType.DMA((1,)),
        ],
        compiler_params=pltpu.CompilerParams(
            vmem_limit_bytes=100 * 1024 * 1024, disable_bounds_checks=True),
    )(x2, w, mean, var, g, b)
    return out.reshape(B, S, C)
```

```python
import jax
import jax.numpy as jnp
from jax import lax
import jax.experimental.pallas as pl
import jax.experimental.pallas.tpu as pltpu

A = 1.6
A2 = A * A
LAM = 0.5 / (A ** 4 - 1.0)
K2 = (A ** 4 + 1.0) / A2
f32 = jnp.float32
u32 = jnp.uint32
bf16 = jnp.bfloat16

TB = 32
TG = 16
NSC = 4
UN = 7
NPK = 40
TGATE = ((0, 56), (1, 56), (2, 56), (3, 56))
SGATE = ((2, 0), (2, 248), (3, 120), (3, 248))
JORD = (1, 2, 3, 4, 0, 5)
SORD = (0, 1, 2, 3, 4, 5)
BORD = (0, 5, 1, 2, 3, 4)


@jax.jit
def pallas_standalone__batchnorm__sampling_kernel(
    x: jax.Array,
    w: jax.Array,
    mean: jax.Array,
    var: jax.Array,
    g: jax.Array,
    b: jax.Array,
):
    B, S, C = x.shape
    assert S == 8 and w.shape == (3, C, C) and C % 128 == 0
    TM = TB * S
    TW = TM // 2
    R = 2 * TB
    RW = R // 2
    NB = C // 128
    NC = B // TB
    NQ = TB // TG
    NG = (NC - NSC) // UN
    assert NB == 5 and NQ == 2 and NSC + NG * UN == NC

    def kernel(x_hbm, w_hbm, mean_hbm, var_hbm, g_hbm, b_hbm, o_hbm,
               xbuf, obuf, wbuf, v_ref, ua_ref, ub_ref, uc_ref, us_ref,
               pb0, pb1, pb2, pb3, p_ref, pk_ref, sx, so, sw, sp):
        pbuf = (pb0, pb1, pb2, pb3)
        one = 1 + pl.program_id(0)

        def xcopies(c0, nch, sem):
            return [pltpu.make_async_copy(
                x_hbm.at[pl.ds(pl.multiple_of(c0 * TM, TM), nch * TM), pl.ds(k * 128, 128)],
                xbuf.at[k, pl.ds(pl.multiple_of(c0 * TW, TW), nch * TW)].bitcast(bf16),
                sx.at[sem]) for k in range(NB)]

        def xgroup(gi):
            return xcopies(NSC + 1 + UN * gi, UN - 1, 3 + 2 * gi)

        def xlast(gi):
            return xcopies(NSC + UN * (gi + 1), 1, 4 + 2 * gi)

        def ocopy(c0, nch, k):
            return pltpu.make_async_copy(
                obuf.at[k, pl.ds(pl.multiple_of(c0 * TW, TW), nch * TW)].bitcast(bf16),
                o_hbm.at[pl.ds(pl.multiple_of(c0 * TM, TM), nch * TM), pl.ds(k * 128, 128)],
                so.at[0])

        def wcopies(n):
            return [pltpu.make_async_copy(
                w_hbm.at[t, :, pl.ds(pl.multiple_of(n * 128, 128), 128)],
                wbuf.at[t, n].bitcast(bf16), sw.at[n]) for t in range(3)]

        pcopies = [pltpu.make_async_copy(h, pbuf[q], sp.at[0])
                   for q, h in enumerate((mean_hbm, var_hbm, g_hbm, b_hbm))]

        def ordered(cps):
            def body(i, c):
                for cp in cps:
                    cp.start()
                return c
            lax.fori_loop(0, one, body, 0)

        def issue_w(n, c):
            for cp in wcopies(n):
                cp.start()
            return c

        def issue_g(gi, c):
            for cp in xgroup(gi):
                cp.start()

            @pl.when(gi + 1 < NG)
            def _():
                for cp in xlast(gi):
                    cp.start()
            return c

        ordered(xcopies(0, 2, 0))
        for cp in pcopies:
            cp.start()
        lax.fori_loop(0, one, issue_w, 0)
        ordered(xcopies(2, 2, 1))
        lax.fori_loop(1, 4, issue_w, 0)
        ordered(xcopies(NSC, 1, 2))
        lax.fori_loop(4, 4 + one, issue_w, 0)
        lax.fori_loop(0, NG, issue_g, 0)

        def zero_from(m):
            return (lax.bitcast_convert_type(m, u32) >> 16) >> 16

        def rep(v, rows):
            return jnp.concatenate([v] * (rows // 8), axis=0)

        def split(lst, pi, npc):
            return lst[pi * len(lst) // npc:(pi + 1) * len(lst) // npc]

        def transform(i, u_ref, pieces, z=None, roff=0):
            if z is None:
                shl = jnp.uint32(16)
                msk = jnp.uint32(0xFFFF0000)
            else:
                shl = rep(z + jnp.uint32(16), TG)
                msk = rep(z + jnp.uint32(0xFFFF0000), TG)
            lo_f32 = lambda w_: lax.bitcast_convert_type(w_ << shl, f32)
            hi_f32 = lambda w_: lax.bitcast_convert_type(w_ & msk, f32)
            for (k, t, q) in pieces:
                cs = slice(k * 128, (k + 1) * 128)
                ev = xbuf[k, pl.ds(i * TW + 4 * q * TG + 2 * t, TG, stride=4), :]
                od = xbuf[k, pl.ds(i * TW + 4 * q * TG + 2 * t + 1, TG, stride=4), :]
                d0 = lo_f32(ev); d1 = hi_f32(ev); d2 = lo_f32(od); d3 = hi_f32(od)
                e1 = d0 + A2 * d2
                o1 = A * d1 + (A * A2) * d3
                e2 = d3 + A2 * d1
                o2 = A * d2 + (A * A2) * d0
                if isinstance(q, int):
                    rr = slice(roff + (t * TB + q * TG) // 2, roff + (t * TB + (q + 1) * TG) // 2)
                else:
                    rr = pl.ds(pl.multiple_of(roff + t * (TB // 2) + q * (TG // 2), 8), TG // 2)
                for j, val in enumerate((d0, e1 + o1, e1 - o1, e2 + o2, e2 - o2, d3)):
                    u_ref.at[j][rr, cs] = pltpu.bitcast(val.astype(bf16), u32)

        def wtransform(n):
            for r in range(C // 32):
                rp = slice(r * 16, (r + 1) * 16)
                ld = lambda t: pltpu.bitcast(wbuf[t, n, rp, :], bf16).astype(f32)
                h0 = ld(2); h1 = ld(1); h2 = ld(0)
                ho = h1 * (LAM * A)
                he = h0 * LAM + h2 * (LAM * A2)
                hr = h2 * LAM + h0 * (LAM * A2)
                for j, val in enumerate((he + ho, he - ho, hr + ho, hr - ho)):
                    v_ref.at[j, n][rp, :] = pltpu.bitcast(val.astype(bf16), u32)

        def vsrc(j, n):
            return wbuf.at[2, n] if j == 0 else wbuf.at[0, n] if j == 5 else v_ref.at[j - 1, n]

        def mm(uval, vval):
            return jnp.dot(pltpu.bitcast(uval, bf16), pltpu.bitcast(vval, bf16),
                           preferred_element_type=f32)

        slot = [0]

        def epi(i, n, Ms):
            scn = rep(p_ref[0, n], TB)
            shn = rep(p_ref[1, n], TB)

            def act(y):
                h = y * scn + shn
                return h + h * jnp.tanh(h)

            for t in range(2):
                a0, Pp, Pm, Qp, Qm, a5 = [Ms[j][t * TB:(t + 1) * TB] for j in range(6)]
                SP = Pp + Pm; DP = Pp - Pm; SQ = Qp + Qm; DQ = Qp - Qm
                b0 = a0 + Ms[0][TB:] if t == 0 else a0
                b5 = a5 + Ms[5][:TB] if t == 1 else a5
                c4 = (SP + b0) - DQ * (1.0 / A)
                c2 = A * DQ - (SP * (1.0 / A2) + a0 * K2)
                c1 = (SQ - DP * (1.0 / A)) + b5
                c3 = (A * DP - SQ * (1.0 / A2)) - a5 * K2
                for pp, (lo, hi) in enumerate(((c1, c2), (c3, c4))):
                    sl = slot[0]
                    slot[0] = (slot[0] + 2) % NPK
                    pk_ref.at[sl][...] = pltpu.bitcast(act(lo).astype(bf16), u32)
                    pk_ref.at[sl + 1][...] = pltpu.bitcast(act(hi).astype(bf16), u32)
                    P = pk_ref[sl]
                    Q = pk_ref[sl + 1]
                    obuf[n, pl.ds(i * TW + 2 * t + pp, TB // 2, stride=8), :] = (
                        (P & jnp.uint32(0xFFFF)) | (Q << 16))
                    obuf[n, pl.ds(i * TW + 4 + 2 * t + pp, TB // 2, stride=8), :] = (
                        (P >> 16) | (Q & jnp.uint32(0xFFFF0000)))

        def epi_multi(c0, ncs, n, Ms):
            for c in range(ncs):
                epi(c0 + c, n, {j: Ms[j][c * R:(c + 1) * R] for j in range(6)})

        allp = [(k, t, q) for k in range(NB) for t in range(2) for q in range(NQ)]
        for cp in xcopies(0, 2, 0):
            cp.wait()
        for c in range(2):
            transform(c, us_ref, allp, roff=c * RW)
        for cp in pcopies:
            cp.wait()
        inv = lax.rsqrt(pbuf[1][...].astype(f32) + 1e-5)
        sc = pbuf[2][...].astype(f32) * inv * 0.5
        sh = pbuf[3][...].astype(f32) * 0.5 - pbuf[0][...].astype(f32) * sc
        sc = sc.reshape(NB, 128)
        sh = sh.reshape(NB, 128)
        for n in range(NB):
            p_ref[0, n] = jnp.broadcast_to(sc[n:n + 1], (8, 128))
            p_ref[1, n] = jnp.broadcast_to(sh[n:n + 1], (8, 128))

        for cp in wcopies(0):
            cp.wait()
        wtransform(0)
        Ms = {j: mm(us_ref[j, 0:2 * RW, :], vsrc(j, 0)[...]) for j in SORD}
        epi_multi(0, 2, 0, Ms)

        for cp in xcopies(2, 2, 1):
            cp.wait()
        for k in range(NB):
            for c in (2, 3):
                transform(c, us_ref, [p for p in allp if p[0] == k], roff=c * RW)
        Ms = {}
        for k in range(NB):
            for j in BORD:
                m = mm(us_ref[j, 2 * RW:4 * RW, k * 128:(k + 1) * 128],
                       vsrc(j, 0)[k * 64:(k + 1) * 64, :])
                Ms[j] = m if k == 0 else Ms[j] + m
        epi_multi(2, 2, 0, Ms)

        def startup(n, carry):
            for cp in wcopies(n):
                cp.wait()

            @pl.when(n == 3)
            def _():
                for cp in xcopies(NSC, 1, 2):
                    cp.wait()

            src = jnp.where(n >= 3, NSC, 0)
            tp = [(k, t, n & 1) for k in range(NB) for t in range(2)]
            wtransform(n)
            Ms = {}
            for pos, j in enumerate(SORD):
                Ms[j] = mm(us_ref[j], vsrc(j, n)[...])
                for gi, (gp, gr) in enumerate(SGATE):
                    if gp == pos:
                        transform(src, ua_ref, split(tp, gi, len(SGATE)),
                                  zero_from(Ms[j][gr:gr + 8]))
            epi_multi(0, NSC, n, Ms)
            return carry

        lax.fori_loop(1, NB, startup, 0)
        for k in range(NB):
            ocopy(0, NSC, k).start()

        def group(gi, carry):
            a = NSC + UN * gi
            for cp in xgroup(gi):
                cp.wait()

            @pl.when(gi + 1 < NG)
            def _():
                for cp in xlast(gi):
                    cp.wait()

            bufs = lambda p: ua_ref if p % UN == 0 else (ub_ref, uc_ref)[p % 2]
            for u in range(UN):
                i = a + u
                inext = jnp.minimum(i + 1, NC - 1)
                ucur, unext = bufs(u), bufs(u + 1)
                for n in range(NB):
                    tp = [(n, t, q) for t in range(2) for q in range(NQ)]
                    Ms = {}
                    for pos, j in enumerate(JORD):
                        Ms[j] = mm(ucur[j], vsrc(j, n)[...])
                        for gi_, (gp, gr) in enumerate(TGATE):
                            if gp == pos:
                                transform(inext, unext, split(tp, gi_, len(TGATE)),
                                          zero_from(Ms[j][gr:gr + 8]))
                    epi(i, n, Ms)
                    ocopy(i, 1, n).start()
            return carry

        lax.fori_loop(0, NG, group, 0)
        pltpu.make_async_copy(o_hbm, o_hbm, so.at[0]).wait()

    anyspec = pl.BlockSpec(memory_space=pl.ANY)
    out = pl.pallas_call(
        kernel,
        grid=(1,),
        in_specs=[anyspec] * 6,
        out_specs=anyspec,
        out_shape=jax.ShapeDtypeStruct((B * S, C), x.dtype),
        scratch_shapes=[
            pltpu.VMEM((NB, B * S // 2, 128), u32),
            pltpu.VMEM((NB, B * S // 2, 128), u32),
            pltpu.VMEM((3, NB, C // 2, 128), u32),
            pltpu.VMEM((4, NB, C // 2, 128), u32),
            pltpu.VMEM((6, RW, C), u32),
            pltpu.VMEM((6, RW, C), u32),
            pltpu.VMEM((6, RW, C), u32),
            pltpu.VMEM((6, NSC * RW, C), u32),
            pltpu.VMEM((C,), bf16), pltpu.VMEM((C,), bf16),
            pltpu.VMEM((C,), bf16), pltpu.VMEM((C,), bf16),
            pltpu.VMEM((2, NB, 8, 128), f32),
            pltpu.VMEM((NPK, TB // 2, 128), u32),
            pltpu.SemaphoreType.DMA((3 + 2 * NG,)),
            pltpu.SemaphoreType.DMA((1,)),
            pltpu.SemaphoreType.DMA((NB,)),
            pltpu.SemaphoreType.DMA((1,)),
        ],
        compiler_params=pltpu.CompilerParams(
            vmem_limit_bytes=100 * 1024 * 1024,
            disable_bounds_checks=True, disable_semaphore_checks=True),
    )(x.reshape(B * S, C), w, mean, var, g, b)
    return out.reshape(B, S, C)
```

```python
import jax
import jax.numpy as jnp
from jax import lax
import jax.experimental.pallas as pl
import jax.experimental.pallas.tpu as pltpu

A = 1.6
A2 = A * A
LAM = 0.5 / (A ** 4 - 1.0)
K2 = (A ** 4 + 1.0) / A2
f32 = jnp.float32
u32 = jnp.uint32
bf16 = jnp.bfloat16

TB = 32
TG = 16
NSC = 4
UN = 7
NPK = 40
TGATE = ((0, 56), (1, 56), (2, 56), (3, 56))
SGATE = ((2, 0), (2, 248), (3, 120), (3, 248))
JORD = (1, 2, 3, 4, 0, 5)
SORD = (0, 1, 2, 3, 4, 5)
BORD = (0, 5, 1, 2, 3, 4)


@jax.jit
def pallas_standalone__batchnorm__sampling_kernel(
    x: jax.Array,
    w: jax.Array,
    mean: jax.Array,
    var: jax.Array,
    g: jax.Array,
    b: jax.Array,
):
    B, S, C = x.shape
    assert S == 8 and w.shape == (3, C, C) and C % 128 == 0
    TM = TB * S
    TW = TM // 2
    R = 2 * TB
    RW = R // 2
    NB = C // 128
    NC = B // TB
    NQ = TB // TG
    NG = (NC - NSC) // UN
    assert NB == 5 and NQ == 2 and NSC + NG * UN == NC

    def kernel(x_hbm, w_hbm, mean_hbm, var_hbm, g_hbm, b_hbm, o_hbm,
               xbuf, obuf, wbuf, v_ref, ua_ref, ub_ref, uc_ref, us_ref,
               pb0, pb1, pb2, pb3, p_ref, pk_ref, sx, so, sw, sp):
        pbuf = (pb0, pb1, pb2, pb3)
        one = 1 + pl.program_id(0)

        def xcopies(c0, nch, sem):
            return [pltpu.make_async_copy(
                x_hbm.at[pl.ds(pl.multiple_of(c0 * TM, TM), nch * TM), pl.ds(k * 128, 128)],
                xbuf.at[k, pl.ds(pl.multiple_of(c0 * TM, TM), nch * TM)],
                sx.at[sem]) for k in range(NB)]

        def xgroup(gi):
            return xcopies(NSC + 1 + UN * gi, UN - 1, 3 + 2 * gi)

        def xlast(gi):
            return xcopies(NSC + UN * (gi + 1), 1, 4 + 2 * gi)

        def ocopy(c0, nch, k):
            return pltpu.make_async_copy(
                obuf.at[k, pl.ds(pl.multiple_of(c0 * TM, TM), nch * TM)],
                o_hbm.at[pl.ds(pl.multiple_of(c0 * TM, TM), nch * TM), pl.ds(k * 128, 128)],
                so.at[0])

        def wcopies(n):
            return [pltpu.make_async_copy(
                w_hbm.at[t, :, pl.ds(pl.multiple_of(n * 128, 128), 128)],
                wbuf.at[t, n], sw.at[n]) for t in range(3)]

        pcopies = [pltpu.make_async_copy(h, pbuf[q], sp.at[0])
                   for q, h in enumerate((mean_hbm, var_hbm, g_hbm, b_hbm))]

        def ordered(cps):
            def body(i, c):
                for cp in cps:
                    cp.start()
                return c
            lax.fori_loop(0, one, body, 0)

        def issue_w(n, c):
            for cp in wcopies(n):
                cp.start()
            return c

        def issue_g(gi, c):
            for cp in xgroup(gi):
                cp.start()

            @pl.when(gi + 1 < NG)
            def _():
                for cp in xlast(gi):
                    cp.start()
            return c

        ordered(xcopies(0, 2, 0))
        for cp in pcopies:
            cp.start()
        lax.fori_loop(0, one, issue_w, 0)
        ordered(xcopies(2, 2, 1))
        lax.fori_loop(1, 4, issue_w, 0)
        ordered(xcopies(NSC, 1, 2))
        lax.fori_loop(4, 4 + one, issue_w, 0)
        lax.fori_loop(0, NG, issue_g, 0)

        xw = xbuf.bitcast(u32)
        ow = obuf.bitcast(u32)
        ww = wbuf.bitcast(u32)

        def zero_from(m):
            return (lax.bitcast_convert_type(m, u32) >> 16) >> 16

        def rep(v, rows):
            return jnp.concatenate([v] * (rows // 8), axis=0)

        def split(lst, pi, npc):
            return lst[pi * len(lst) // npc:(pi + 1) * len(lst) // npc]

        def transform(i, u_ref, pieces, z=None, roff=0):
            if z is None:
                shl = jnp.uint32(16)
                msk = jnp.uint32(0xFFFF0000)
            else:
                shl = rep(z + jnp.uint32(16), TG)
                msk = rep(z + jnp.uint32(0xFFFF0000), TG)
            lo_f32 = lambda w_: lax.bitcast_convert_type(w_ << shl, f32)
            hi_f32 = lambda w_: lax.bitcast_convert_type(w_ & msk, f32)
            for (k, t, q) in pieces:
                cs = slice(k * 128, (k + 1) * 128)
                xv = xw.at[k, pl.ds(pl.multiple_of(i * TW + 4 * q * TG, 4 * TG), 4 * TG)]
                ev = xv[pl.ds(2 * t, TG, stride=4), :]
                od = xv[pl.ds(2 * t + 1, TG, stride=4), :]
                d0 = lo_f32(ev); d1 = hi_f32(ev); d2 = lo_f32(od); d3 = hi_f32(od)
                e1 = d0 + A2 * d2
                o1 = A * d1 + (A * A2) * d3
                e2 = d3 + A2 * d1
                o2 = A * d2 + (A * A2) * d0
                if isinstance(q, int):
                    rr = slice(roff + (t * TB + q * TG) // 2, roff + (t * TB + (q + 1) * TG) // 2)
                else:
                    rr = pl.ds(pl.multiple_of(roff + t * (TB // 2) + q * (TG // 2), 8), TG // 2)
                for j, val in enumerate((d0, e1 + o1, e1 - o1, e2 + o2, e2 - o2, d3)):
                    u_ref.at[j][rr, cs] = pltpu.bitcast(val.astype(bf16), u32)

        def wtransform(n):
            for r in range(C // 32):
                rp = slice(r * 16, (r + 1) * 16)
                ld = lambda t: pltpu.bitcast(ww[t, n, rp, :], bf16).astype(f32)
                h0 = ld(2); h1 = ld(1); h2 = ld(0)
                ho = h1 * (LAM * A)
                he = h0 * LAM + h2 * (LAM * A2)
                hr = h2 * LAM + h0 * (LAM * A2)
                for j, val in enumerate((he + ho, he - ho, hr + ho, hr - ho)):
                    v_ref.at[j, n][rp, :] = pltpu.bitcast(val.astype(bf16), u32)

        def vsrc(j, n):
            return ww.at[2, n] if j == 0 else ww.at[0, n] if j == 5 else v_ref.at[j - 1, n]

        def mm(uval, vval):
            return jnp.dot(pltpu.bitcast(uval, bf16), pltpu.bitcast(vval, bf16),
                           preferred_element_type=f32)

        slot = [0]

        def epi(i, n, Ms):
            scn = rep(p_ref[0, n], TB)
            shn = rep(p_ref[1, n], TB)

            def act(y):
                h = y * scn + shn
                return h + h * jnp.tanh(h)

            ov = ow.at[n, pl.ds(pl.multiple_of(i * TW, TW), TW)]
            for t in range(2):
                a0, Pp, Pm, Qp, Qm, a5 = [Ms[j][t * TB:(t + 1) * TB] for j in range(6)]
                SP = Pp + Pm; DP = Pp - Pm; SQ = Qp + Qm; DQ = Qp - Qm
                b0 = a0 + Ms[0][TB:] if t == 0 else a0
                b5 = a5 + Ms[5][:TB] if t == 1 else a5
                c4 = (SP + b0) - DQ * (1.0 / A)
                c2 = A * DQ - (SP * (1.0 / A2) + a0 * K2)
                c1 = (SQ - DP * (1.0 / A)) + b5
                c3 = (A * DP - SQ * (1.0 / A2)) - a5 * K2
                for pp, (lo, hi) in enumerate(((c1, c2), (c3, c4))):
                    sl = slot[0]
                    slot[0] = (slot[0] + 2) % NPK
                    pk_ref.at[sl][...] = pltpu.bitcast(act(lo).astype(bf16), u32)
                    pk_ref.at[sl + 1][...] = pltpu.bitcast(act(hi).astype(bf16), u32)
                    P = pk_ref[sl]
                    Q = pk_ref[sl + 1]
                    ov[pl.ds(2 * t + pp, TB // 2, stride=8), :] = (
                        (P & jnp.uint32(0xFFFF)) | (Q << 16))
                    ov[pl.ds(4 + 2 * t + pp, TB // 2, stride=8), :] = (
                        (P >> 16) | (Q & jnp.uint32(0xFFFF0000)))

        def epi_multi(c0, ncs, n, Ms):
            for c in range(ncs):
                epi(c0 + c, n, {j: Ms[j][c * R:(c + 1) * R] for j in range(6)})

        allp = [(k, t, q) for k in range(NB) for t in range(2) for q in range(NQ)]
        for cp in xcopies(0, 2, 0):
            cp.wait()
        for c in range(2):
            transform(c, us_ref, allp, roff=c * RW)
        for cp in pcopies:
            cp.wait()
        inv = lax.rsqrt(pbuf[1][...].astype(f32) + 1e-5)
        sc = pbuf[2][...].astype(f32) * inv * 0.5
        sh = pbuf[3][...].astype(f32) * 0.5 - pbuf[0][...].astype(f32) * sc
        sc = sc.reshape(NB, 128)
        sh = sh.reshape(NB, 128)
        for n in range(NB):
            p_ref[0, n] = jnp.broadcast_to(sc[n:n + 1], (8, 128))
            p_ref[1, n] = jnp.broadcast_to(sh[n:n + 1], (8, 128))

        for cp in wcopies(0):
            cp.wait()
        wtransform(0)
        Ms = {j: mm(us_ref[j, 0:2 * RW, :], vsrc(j, 0)[...]) for j in SORD}
        epi_multi(0, 2, 0, Ms)

        for cp in xcopies(2, 2, 1):
            cp.wait()
        for k in range(NB):
            for c in (2, 3):
                transform(c, us_ref, [p for p in allp if p[0] == k], roff=c * RW)
        Ms = {}
        for k in range(NB):
            for j in BORD:
                m = mm(us_ref[j, 2 * RW:4 * RW, k * 128:(k + 1) * 128],
                       vsrc(j, 0)[k * 64:(k + 1) * 64, :])
                Ms[j] = m if k == 0 else Ms[j] + m
        epi_multi(2, 2, 0, Ms)

        def startup(n, carry):
            for cp in wcopies(n):
                cp.wait()

            @pl.when(n == 3)
            def _():
                for cp in xcopies(NSC, 1, 2):
                    cp.wait()

            src = jnp.where(n >= 3, NSC, 0)
            tp = [(k, t, n & 1) for k in range(NB) for t in range(2)]
            wtransform(n)
            Ms = {}
            for pos, j in enumerate(SORD):
                Ms[j] = mm(us_ref[j], vsrc(j, n)[...])
                for gi, (gp, gr) in enumerate(SGATE):
                    if gp == pos:
                        transform(src, ua_ref, split(tp, gi, len(SGATE)),
                                  zero_from(Ms[j][gr:gr + 8]))
            epi_multi(0, NSC, n, Ms)
            return carry

        lax.fori_loop(1, NB, startup, 0)
        for k in range(NB):
            ocopy(0, NSC, k).start()

        def group(gi, carry):
            a = NSC + UN * gi
            for cp in xgroup(gi):
                cp.wait()

            @pl.when(gi + 1 < NG)
            def _():
                for cp in xlast(gi):
                    cp.wait()

            bufs = lambda p: ua_ref if p % UN == 0 else (ub_ref, uc_ref)[p % 2]
            for u in range(UN):
                i = a + u
                inext = jnp.minimum(i + 1, NC - 1)
                ucur, unext = bufs(u), bufs(u + 1)
                for n in range(NB):
                    tp = [(n, t, q) for t in range(2) for q in range(NQ)]
                    Ms = {}
                    for pos, j in enumerate(JORD):
                        Ms[j] = mm(ucur[j], vsrc(j, n)[...])
                        for gi_, (gp, gr) in enumerate(TGATE):
                            if gp == pos:
                                transform(inext, unext, split(tp, gi_, len(TGATE)),
                                          zero_from(Ms[j][gr:gr + 8]))
                    epi(i, n, Ms)
                    ocopy(i, 1, n).start()
            return carry

        lax.fori_loop(0, NG, group, 0)
        pltpu.make_async_copy(o_hbm, o_hbm, so.at[0]).wait()

    anyspec = pl.BlockSpec(memory_space=pl.ANY)
    out = pl.pallas_call(
        kernel,
        grid=(1,),
        in_specs=[anyspec] * 6,
        out_specs=anyspec,
        out_shape=jax.ShapeDtypeStruct((B * S, C), x.dtype),
        scratch_shapes=[
            pltpu.VMEM((NB, B * S, 128), bf16),
            pltpu.VMEM((NB, B * S, 128), bf16),
            pltpu.VMEM((3, NB, C, 128), bf16),
            pltpu.VMEM((4, NB, C // 2, 128), u32),
            pltpu.VMEM((6, RW, C), u32),
            pltpu.VMEM((6, RW, C), u32),
            pltpu.VMEM((6, RW, C), u32),
            pltpu.VMEM((6, NSC * RW, C), u32),
            pltpu.VMEM((C,), bf16), pltpu.VMEM((C,), bf16),
            pltpu.VMEM((C,), bf16), pltpu.VMEM((C,), bf16),
            pltpu.VMEM((2, NB, 8, 128), f32),
            pltpu.VMEM((NPK, TB // 2, 128), u32),
            pltpu.SemaphoreType.DMA((3 + 2 * NG,)),
            pltpu.SemaphoreType.DMA((1,)),
            pltpu.SemaphoreType.DMA((NB,)),
            pltpu.SemaphoreType.DMA((1,)),
        ],
        compiler_params=pltpu.CompilerParams(
            vmem_limit_bytes=100 * 1024 * 1024,
            disable_bounds_checks=True, disable_semaphore_checks=True),
    )(x.reshape(B * S, C), w, mean, var, g, b)
    return out.reshape(B, S, C)
```

```python
import jax
import jax.numpy as jnp
from jax import lax
import jax.experimental.pallas as pl
import jax.experimental.pallas.tpu as pltpu

f32 = jnp.float32
u32 = jnp.uint32
bf16 = jnp.bfloat16

NJ = 11
KQ = 0.5 / 225.0
TB = 64
TG = 16
NSC = 2
UN = 2
XPRE = 3
NPK = 40

_N = (None, 0)
JORD = (9, 10, 5, 6, 2, 7, 8, 4, 1, 3, 0)
TGATE = ((0, 24), (2, 0), (6, 0), (7, 0))
W1G = (_N,) * 8 + tuple((p, r) for p in range(3) for r in (24, 56, 88, 120))
SORD = (7, 8, 9, 10, 5, 6, 3, 0, 4, 1, 2)
SGATE = (_N,) * 5 + tuple((p, r) for p in range(5) for r in (24, 72, 120))
FORD = (7, 8, 9, 10, 5, 6, 3, 4)
FGATE = ((_N,) * 5 + tuple((p, r) for p in range(5) for r in (24, 56))
         + tuple((p, 56) for p in (10, 11, 12, 13, 9)))


@jax.jit
def pallas_standalone__batchnorm__sampling_kernel(
    x: jax.Array,
    w: jax.Array,
    mean: jax.Array,
    var: jax.Array,
    g: jax.Array,
    b: jax.Array,
):
    B, S, C = x.shape
    assert S == 8 and w.shape == (3, C, C) and C == 5 * 128
    TM = TB * S
    TW = TM // 2
    RW = TB // 2
    NB = C // 128
    NC = B // TB
    NQ = TB // TG
    NG = (NC - NSC) // UN
    NR = C // 32
    assert NSC + NG * UN == NC and XPRE < NG

    def kernel(x_hbm, w_hbm, mean_hbm, var_hbm, g_hbm, b_hbm, o_hbm,
               xbuf, obuf, wbuf, v_ref, ua_ref, ub_ref, us_ref, mr_ref,
               pb0, pb1, pb2, pb3, p_ref, pk_ref, sx, so, sw, sp):
        pbuf = (pb0, pb1, pb2, pb3)
        one = 1 + pl.program_id(0)

        def xcopies(c):
            return [pltpu.make_async_copy(
                x_hbm.at[pl.ds(pl.multiple_of(c * TM, TM), TM), pl.ds(k * 128, 128)],
                xbuf.at[k, pl.ds(pl.multiple_of(c * TM, TM), TM)],
                sx.at[c]) for k in range(NB)]

        def ocopy(r0, nrows, k):
            return pltpu.make_async_copy(
                obuf.at[k, pl.ds(pl.multiple_of(r0, TM // 2), nrows)],
                o_hbm.at[pl.ds(pl.multiple_of(r0, TM // 2), nrows), pl.ds(k * 128, 128)],
                so.at[0])

        def wcopies(n):
            return [pltpu.make_async_copy(
                w_hbm.at[t, :, pl.ds(pl.multiple_of(n * 128, 128), 128)],
                wbuf.at[t, n], sw.at[n]) for t in range(3)]

        pcopies = [pltpu.make_async_copy(h, pbuf[q], sp.at[0])
                   for q, h in enumerate((mean_hbm, var_hbm, g_hbm, b_hbm))]

        def issue_w(n, carry):
            for cp in wcopies(n):
                cp.start()
            return carry

        def issue_x(c, carry):
            for cp in xcopies(c):
                cp.start()
            return carry

        for cp in pcopies:
            cp.start()
        lax.fori_loop(0, one, issue_w, 0)
        lax.fori_loop(0, NSC, issue_x, 0)
        lax.fori_loop(1, NB, issue_w, 0)
        lax.fori_loop(NSC, NSC + 1 + UN * XPRE, issue_x, 0)

        xw = xbuf.bitcast(u32)
        ow = obuf.bitcast(u32)
        ww = wbuf.bitcast(u32)

        def zero_from(m):
            return (lax.bitcast_convert_type(m, u32) >> 16) >> 16

        def rep(v, rows):
            return jnp.concatenate([v] * (rows // 8), axis=0)

        def split(lst, pi, npc):
            return lst[pi * len(lst) // npc:(pi + 1) * len(lst) // npc]

        def transform(i, u_ref, pieces, z=None):
            if z is None:
                shl = jnp.uint32(16)
                msk = jnp.uint32(0xFFFF0000)
            else:
                shl = rep(z + jnp.uint32(16), TG)
                msk = rep(z + jnp.uint32(0xFFFF0000), TG)
            for (k, q) in pieces:
                xv = xw.at[k, pl.ds(pl.multiple_of(i * TW + 4 * q * TG, 4 * TG), 4 * TG)]
                d = []
                for p in range(4):
                    wv = xv[pl.ds(p, TG, stride=4), :]
                    d.append(lax.bitcast_convert_type(wv << shl, f32))
                    d.append(lax.bitcast_convert_type(wv & msk, f32))
                s04 = d[0] + d[4]; s26 = d[2] + d[6]; s15 = d[1] + d[5]; s37 = d[3] + d[7]
                e1 = s04 + s26; xr = s04 - s26; o1 = s15 + s37; xi = s15 - s37
                e4 = (d[0] + 16.0 * d[4]) + 4.0 * (d[2] + 16.0 * d[6])
                o4 = 2.0 * ((d[1] + 16.0 * d[5]) + 4.0 * (d[3] + 16.0 * d[7]))
                f4 = (d[7] + 16.0 * d[3]) + 4.0 * (d[5] + 16.0 * d[1])
                g4 = 2.0 * ((d[6] + 16.0 * d[2]) + 4.0 * (d[4] + 16.0 * d[0]))
                vals = (d[0], d[7], xr + xi, xr, xi, e1 + o1, e1 - o1,
                        e4 + o4, e4 - o4, f4 + g4, f4 - g4)
                rr = slice(q * TG // 2, (q + 1) * TG // 2)
                cs = slice(k * 128, (k + 1) * 128)
                for j, val in enumerate(vals):
                    u_ref.at[j][rr, cs] = pltpu.bitcast(val.astype(bf16), u32)

        def wtransform(n, vdst, rows, z=None):
            zz = None if z is None else rep(z, 16)
            for r in rows:
                rp = slice(r * 16, (r + 1) * 16)

                def ld(t):
                    wv = ww[t, n, rp, :]
                    if zz is not None:
                        wv = wv + zz
                    return pltpu.bitcast(wv, bf16).astype(f32)

                h0 = ld(2); h1 = ld(1); h2 = ld(0)
                c = h0 - h2
                hs = (h0 + h2) * 0.5
                hh = h1 * 0.5
                bq = h1 * (2 * KQ)
                aq = h0 * KQ + h2 * (4 * KQ)
                ar = h2 * KQ + h0 * (4 * KQ)
                vals = (c + h1, c - h1, hs + hh, hs - hh, aq + bq, aq - bq, ar + bq, ar - bq)
                for j, val in enumerate(vals):
                    vdst.at[j // 2][rp, (j % 2) * 128:(j % 2 + 1) * 128] = (
                        pltpu.bitcast(val.astype(bf16), u32))

        def vsrc(j, n, vv=None):
            if j < 3:
                return ww.at[(2, 0, 1)[j], n]
            vv = v_ref.at[n] if vv is None else vv
            return vv.at[(j - 3) // 2, :, ((j - 3) % 2) * 128:((j - 3) % 2 + 1) * 128]

        def mm(uval, vval):
            return jnp.dot(pltpu.bitcast(uval, bf16), pltpu.bitcast(vval, bf16),
                           preferred_element_type=f32)

        slot = [0]

        def epi(i, n, Ms):
            scn = rep(p_ref[0, n], TB)
            shn = rep(p_ref[1, n], TB)

            def act(y):
                h = y * scn + shn
                return h + h * jnp.tanh(h)

            def solve(a1, a2, a3, a4, e0):
                s2 = a1 + a2; d2 = a1 - a2
                hq = 0.5 * a4
                ap = a3 + hq; am = a3 - hq
                t1 = ap - (34.0 / 225.0) * d2
                tau = t1 - (16.0 / 225.0) * s2
                e2 = (0.5 + 16.0 / 225.0) * s2 - t1
                e4 = tau - e0
                rh = (225.0 / 120.0) * am - 2.125 * (e4 - e0)
                dq = 0.25 * d2
                return dq - rh, e2, dq + rh, e4

            m0, m9, k1, k2, k3, Pp, Pm, Qp, Qm, Rp, Rm = [Ms[j] for j in range(NJ)]
            c2, c4, c6, c8 = solve(Pp + Pm, k2 - k1, Qp + Qm, Rp - Rm, m0)
            c7, c5, c3, c1 = solve(Pp - Pm, k3 + k1, Rp + Rm, Qp - Qm, m9)
            ov = ow.at[n, pl.ds(pl.multiple_of(i * TW, TW), TW)]
            for pp, (lo, hi) in enumerate(((c1, c2), (c3, c4), (c5, c6), (c7, c8))):
                sl = slot[0]
                slot[0] = (slot[0] + 1) % NPK
                pk_ref.at[sl][:, 0:128] = pltpu.bitcast(act(lo).astype(bf16), u32)
                pk_ref.at[sl][:, 128:256] = pltpu.bitcast(act(hi).astype(bf16), u32)
                P = pk_ref[sl, :, 0:128]
                Q = pk_ref[sl, :, 128:256]
                ov[pl.ds(pp, TB // 2, stride=8), :] = (P & jnp.uint32(0xFFFF)) | (Q << 16)
                ov[pl.ds(4 + pp, TB // 2, stride=8), :] = (
                    (P >> 16) | (Q & jnp.uint32(0xFFFF0000)))

        allp = [(k, q) for k in range(NB) for q in range(NQ)]
        allr = list(range(NR))

        for cp in pcopies:
            cp.wait()
        inv = lax.rsqrt(pbuf[1][...].astype(f32) + 1e-5)
        sc = pbuf[2][...].astype(f32) * inv * 0.5
        sh = pbuf[3][...].astype(f32) * 0.5 - pbuf[0][...].astype(f32) * sc
        sc = sc.reshape(NB, 128)
        sh = sh.reshape(NB, 128)
        for n in range(NB):
            p_ref[0, n] = jnp.broadcast_to(sc[n:n + 1], (8, 128))
            p_ref[1, n] = jnp.broadcast_to(sh[n:n + 1], (8, 128))
        for cp in wcopies(0):
            cp.wait()
        wtransform(0, v_ref.at[0], allr)

        def first_block(c, carry):
            for cp in xcopies(c):
                cp.wait()
            usv = us_ref.at[:, pl.ds(pl.multiple_of(c * RW, RW), RW), :]
            transform(c, usv, allp)
            Ms = {}
            for k in range(NB):
                for j in range(NJ):
                    m = mm(usv[j, :, k * 128:(k + 1) * 128], vsrc(j, 0)[k * 64:(k + 1) * 64, :])
                    Ms[j] = m if k == 0 else Ms[j] + m
            epi(c, 0, Ms)
            return carry

        lax.fori_loop(0, NSC, first_block, 0)

        for cp in wcopies(1):
            cp.wait()
        for gi, (gp, gr) in enumerate(W1G):
            if gp is None:
                wtransform(1, v_ref.at[1], split(allr, gi, len(W1G)))
        for j in range(3):
            m = mm(us_ref[j], vsrc(j, 1)[...])
            mr_ref[j] = m
            for gi, (gp, gr) in enumerate(W1G):
                if gp == j:
                    wtransform(1, v_ref.at[1], split(allr, gi, len(W1G)),
                               zero_from(m[gr:gr + 8]))

        def step(r, carry):
            for cp in wcopies(r):
                cp.wait()
            v2 = v_ref.at[pl.ds(r - 1, 2)]
            for gi, (gp, gr) in enumerate(SGATE):
                if gp is None:
                    wtransform(r, v2.at[1], split(allr, gi, len(SGATE)))
            Ms = {j: mr_ref[j] for j in range(3)}
            raws = {}
            for pos, j in enumerate(SORD):
                if j < 3:
                    m = raws[j] = mm(us_ref[j], vsrc(j, r)[...])
                else:
                    m = Ms[j] = mm(us_ref[j], vsrc(j, r - 1, v2.at[0])[...])
                for gi, (gp, gr) in enumerate(SGATE):
                    if gp == pos:
                        wtransform(r, v2.at[1], split(allr, gi, len(SGATE)),
                                   zero_from(m[gr:gr + 8]))
            for c in range(NSC):
                epi(c, r - 1, {j: Ms[j][c * TB:(c + 1) * TB] for j in range(NJ)})
            for j in range(3):
                mr_ref[j] = raws[j]
            return carry

        lax.fori_loop(2, NB, step, 0)

        for cp in xcopies(NSC):
            cp.wait()
        for gi, (gp, gr) in enumerate(FGATE):
            if gp is None:
                transform(NSC, ua_ref, split(allp, gi, len(FGATE)))
        for c in range(NSC):
            Ms = {j: mr_ref[j, c * TB:(c + 1) * TB] for j in range(3)}
            for pos, j in enumerate(FORD):
                Ms[j] = mm(us_ref[j, c * RW:(c + 1) * RW, :], vsrc(j, NB - 1)[...])
                for gi, (gp, gr) in enumerate(FGATE):
                    if gp == pos + len(FORD) * c:
                        transform(NSC, ua_ref, split(allp, gi, len(FGATE)),
                                  zero_from(Ms[j][gr:gr + 8]))
            epi(c, NB - 1, Ms)
        for k in range(NB):
            ocopy(0, NSC * TM, k).start()

        def group(gi, carry):
            a = NSC + UN * gi
            for cp in xcopies(a + 1):
                cp.wait()

            @pl.when(a + 2 < NC)
            def _():
                for cp in xcopies(a + 2):
                    cp.wait()

            for u in range(UN):
                i = a + u
                inext = jnp.minimum(i + 1, NC - 1)
                ucur, unext = (ua_ref, ub_ref) if u == 0 else (ub_ref, ua_ref)
                for n in range(NB):
                    Ms = {}
                    for pos, j in enumerate(JORD):
                        Ms[j] = mm(ucur[j], vsrc(j, n)[...])
                        for q, (gp, gr) in enumerate(TGATE):
                            if gp == pos:
                                transform(inext, unext, [(n, q)], zero_from(Ms[j][gr:gr + 8]))
                    epi(i, n, Ms)
                    ocopy(i * TM, TM, n).start()
            for d in range(UN):
                @pl.when(a + 1 + UN * XPRE + d < NC)
                def _():
                    issue_x(a + 1 + UN * XPRE + d, 0)
            return carry

        lax.fori_loop(0, NG, group, 0)
        pltpu.make_async_copy(o_hbm, o_hbm, so.at[0]).wait()

    anyspec = pl.BlockSpec(memory_space=pl.ANY)
    out = pl.pallas_call(
        kernel,
        grid=(1,),
        in_specs=[anyspec] * 6,
        out_specs=anyspec,
        out_shape=jax.ShapeDtypeStruct((B * S, C), x.dtype),
        scratch_shapes=[
            pltpu.VMEM((NB, B * S, 128), bf16),
            pltpu.VMEM((NB, B * S, 128), bf16),
            pltpu.VMEM((3, NB, C, 128), bf16),
            pltpu.VMEM((NB, 4, C // 2, 256), u32),
            pltpu.VMEM((NJ, RW, C), u32),
            pltpu.VMEM((NJ, RW, C), u32),
            pltpu.VMEM((NJ, NSC * RW, C), u32),
            pltpu.VMEM((3, NSC * TB, 128), f32),
            pltpu.VMEM((C,), bf16), pltpu.VMEM((C,), bf16),
            pltpu.VMEM((C,), bf16), pltpu.VMEM((C,), bf16),
            pltpu.VMEM((2, NB, 8, 128), f32),
            pltpu.VMEM((NPK, TB // 2, 256), u32),
            pltpu.SemaphoreType.DMA((NC,)),
            pltpu.SemaphoreType.DMA((1,)),
            pltpu.SemaphoreType.DMA((NB,)),
            pltpu.SemaphoreType.DMA((1,)),
        ],
        compiler_params=pltpu.CompilerParams(
            vmem_limit_bytes=100 * 1024 * 1024,
            disable_bounds_checks=True, disable_semaphore_checks=True),
    )(x.reshape(B * S, C), w, mean, var, g, b)
    return out.reshape(B, S, C)
```

```python
import jax
import jax.numpy as jnp
from jax import lax
import jax.experimental.pallas as pl
import jax.experimental.pallas.tpu as pltpu

f32 = jnp.float32
u32 = jnp.uint32
bf16 = jnp.bfloat16

NJ = 11
KQ = 0.5 / 225.0
TB = 64
TG = 16
NSC = 2
UN = 2
XPRE = 3
NPK = 40

_N = (None, 0)
JORD = (5, 6, 9, 10, 2, 7, 8, 4, 1, 3, 0)
TGATE = ((1, 0), (2, 24), (5, 0), (7, 0))
W1G = (_N,) * 8 + tuple((p, r) for p in range(3) for r in (24, 56, 88, 120))
SORD = (7, 8, 9, 10, 5, 6, 3, 0, 4, 1, 2)
SGATE = (_N,) * 5 + tuple((p, r) for p in range(5) for r in (24, 72, 120))
FORD = (7, 8, 9, 10, 5, 6, 3, 4)
FGATE = ((_N,) * 5 + tuple((p, r) for p in range(5) for r in (24, 56))
         + tuple((p, 56) for p in (10, 11, 12, 13, 9)))


def _compiler_params():
    kw = dict(vmem_limit_bytes=100 * 1024 * 1024, disable_bounds_checks=True)
    try:
        return pltpu.CompilerParams(disable_semaphore_checks=True, **kw)
    except TypeError:
        return pltpu.CompilerParams(**kw)


@jax.jit
def pallas_standalone__batchnorm__sampling_kernel(
    x: jax.Array,
    w: jax.Array,
    mean: jax.Array,
    var: jax.Array,
    g: jax.Array,
    b: jax.Array,
):
    B, S, C = x.shape
    assert S == 8 and w.shape == (3, C, C) and C == 5 * 128
    TM = TB * S
    TW = TM // 2
    RW = TB // 2
    NB = C // 128
    NC = B // TB
    NQ = TB // TG
    NG = (NC - NSC) // UN
    NR = C // 32
    assert NSC + NG * UN == NC and XPRE < NG

    def kernel(x_hbm, w_hbm, mean_hbm, var_hbm, g_hbm, b_hbm, o_hbm,
               xbuf, obuf, wbuf, v_ref, ua_ref, ub_ref, us_ref, mr_ref,
               pb0, pb1, pb2, pb3, p_ref, pk_ref, sx, so, sw, sp):
        pbuf = (pb0, pb1, pb2, pb3)
        one = 1 + pl.program_id(0)

        def xcopies(c):
            return [pltpu.make_async_copy(
                x_hbm.at[pl.ds(pl.multiple_of(c * TM, TM), TM), pl.ds(k * 128, 128)],
                xbuf.at[k, pl.ds(pl.multiple_of(c * TM, TM), TM)],
                sx.at[c]) for k in range(NB)]

        def ocopy(r0, nrows, k):
            return pltpu.make_async_copy(
                obuf.at[k, pl.ds(pl.multiple_of(r0, TM), nrows)],
                o_hbm.at[pl.ds(pl.multiple_of(r0, TM), nrows), pl.ds(k * 128, 128)],
                so.at[0])

        def wcopies(n):
            return [pltpu.make_async_copy(
                w_hbm.at[t, :, pl.ds(pl.multiple_of(n * 128, 128), 128)],
                wbuf.at[t, n], sw.at[n]) for t in range(3)]

        pcopies = [pltpu.make_async_copy(h, pbuf[q], sp.at[0])
                   for q, h in enumerate((mean_hbm, var_hbm, g_hbm, b_hbm))]

        def issue_w(n, carry):
            for cp in wcopies(n):
                cp.start()
            return carry

        def issue_x(c, carry):
            for cp in xcopies(c):
                cp.start()
            return carry

        for cp in pcopies:
            cp.start()
        lax.fori_loop(0, one, issue_w, 0)
        lax.fori_loop(0, NSC, issue_x, 0)
        lax.fori_loop(1, NB, issue_w, 0)
        lax.fori_loop(NSC, NSC + 1 + UN * XPRE, issue_x, 0)

        xw = xbuf.bitcast(u32)
        ow = obuf.bitcast(u32)
        ww = wbuf.bitcast(u32)

        def zero_from(m):
            return (lax.bitcast_convert_type(m, u32) >> 16) >> 16

        def rep(v, rows):
            return jnp.concatenate([v] * (rows // 8), axis=0)

        def split(lst, pi, npc):
            return lst[pi * len(lst) // npc:(pi + 1) * len(lst) // npc]

        def transform(i, u_ref, pieces, z=None):
            if z is None:
                shl = jnp.uint32(16)
                msk = jnp.uint32(0xFFFF0000)
            else:
                shl = rep(z + jnp.uint32(16), TG)
                msk = rep(z + jnp.uint32(0xFFFF0000), TG)
            for (k, q) in pieces:
                xv = xw.at[k, pl.ds(pl.multiple_of(i * TW + 4 * q * TG, 4 * TG), 4 * TG)]
                d = []
                for p in range(4):
                    wv = xv[pl.ds(p, TG, stride=4), :]
                    d.append(lax.bitcast_convert_type(wv << shl, f32))
                    d.append(lax.bitcast_convert_type(wv & msk, f32))
                s04 = d[0] + d[4]; s26 = d[2] + d[6]; s15 = d[1] + d[5]; s37 = d[3] + d[7]
                e1 = s04 + s26; xr = s04 - s26; o1 = s15 + s37; xi = s15 - s37
                e4 = (d[0] + 16.0 * d[4]) + 4.0 * (d[2] + 16.0 * d[6])
                o4 = 2.0 * ((d[1] + 16.0 * d[5]) + 4.0 * (d[3] + 16.0 * d[7]))
                f4 = (d[7] + 16.0 * d[3]) + 4.0 * (d[5] + 16.0 * d[1])
                g4 = 2.0 * ((d[6] + 16.0 * d[2]) + 4.0 * (d[4] + 16.0 * d[0]))
                vals = (d[0], d[7], xr + xi, xr, xi, e1 + o1, e1 - o1,
                        e4 + o4, e4 - o4, f4 + g4, f4 - g4)
                rr = slice(q * TG // 2, (q + 1) * TG // 2)
                cs = slice(k * 128, (k + 1) * 128)
                for j, val in enumerate(vals):
                    u_ref.at[j][rr, cs] = pltpu.bitcast(val.astype(bf16), u32)

        def wtransform(n, vdst, rows, z=None):
            zz = None if z is None else rep(z, 16)
            for r in rows:
                rp = slice(r * 16, (r + 1) * 16)

                def ld(t):
                    wv = ww[t, n, rp, :]
                    if zz is not None:
                        wv = wv + zz
                    return pltpu.bitcast(wv, bf16).astype(f32)

                h0 = ld(2); h1 = ld(1); h2 = ld(0)
                c = h0 - h2
                hs = (h0 + h2) * 0.5
                hh = h1 * 0.5
                bq = h1 * (2 * KQ)
                aq = h0 * KQ + h2 * (4 * KQ)
                ar = h2 * KQ + h0 * (4 * KQ)
                vals = (c + h1, c - h1, hs + hh, hs - hh, aq + bq, aq - bq, ar + bq, ar - bq)
                for j, val in enumerate(vals):
                    vdst.at[j // 2][rp, (j % 2) * 128:(j % 2 + 1) * 128] = (
                        pltpu.bitcast(val.astype(bf16), u32))

        def vsrc(j, n, vv=None):
            if j < 3:
                return ww.at[(2, 0, 1)[j], n]
            vv = v_ref.at[n] if vv is None else vv
            return vv.at[(j - 3) // 2, :, ((j - 3) % 2) * 128:((j - 3) % 2 + 1) * 128]

        def mm(uval, vval):
            return jnp.dot(pltpu.bitcast(uval, bf16), pltpu.bitcast(vval, bf16),
                           preferred_element_type=f32)

        slot = [0]

        def epi(i, n, Ms):
            scn = rep(p_ref[0, n], TB)
            shn = rep(p_ref[1, n], TB)

            def act(y):
                h = y * scn + shn
                return h + h * jnp.tanh(h)

            def solve(a1, a2, a3, a4, e0):
                s2 = a1 + a2; d2 = a1 - a2
                hq = 0.5 * a4
                ap = a3 + hq; am = a3 - hq
                t1 = ap - (34.0 / 225.0) * d2
                tau = t1 - (16.0 / 225.0) * s2
                e2 = (0.5 + 16.0 / 225.0) * s2 - t1
                e4 = tau - e0
                rh = (225.0 / 120.0) * am - 2.125 * (e4 - e0)
                dq = 0.25 * d2
                return dq - rh, e2, dq + rh, e4

            m0, m9, k1, k2, k3, Pp, Pm, Qp, Qm, Rp, Rm = [Ms[j] for j in range(NJ)]
            c2, c4, c6, c8 = solve(Pp + Pm, k2 - k1, Qp + Qm, Rp - Rm, m0)
            c7, c5, c3, c1 = solve(Pp - Pm, k3 + k1, Rp + Rm, Qp - Qm, m9)
            ov = ow.at[n, pl.ds(pl.multiple_of(i * TW, TW), TW)]
            for pp, (lo, hi) in enumerate(((c1, c2), (c3, c4), (c5, c6), (c7, c8))):
                sl = slot[0]
                slot[0] = (slot[0] + 1) % NPK
                pk_ref.at[sl][:, 0:128] = pltpu.bitcast(act(lo).astype(bf16), u32)
                pk_ref.at[sl][:, 128:256] = pltpu.bitcast(act(hi).astype(bf16), u32)
                P = pk_ref[sl, :, 0:128]
                Q = pk_ref[sl, :, 128:256]
                ov[pl.ds(pp, TB // 2, stride=8), :] = (P & jnp.uint32(0xFFFF)) | (Q << 16)
                ov[pl.ds(4 + pp, TB // 2, stride=8), :] = (
                    (P >> 16) | (Q & jnp.uint32(0xFFFF0000)))

        allp = [(k, q) for k in range(NB) for q in range(NQ)]
        allr = list(range(NR))

        for cp in pcopies:
            cp.wait()
        inv = lax.rsqrt(pbuf[1][...].astype(f32) + 1e-5)
        sc = pbuf[2][...].astype(f32) * inv * 0.5
        sh = pbuf[3][...].astype(f32) * 0.5 - pbuf[0][...].astype(f32) * sc
        sc = sc.reshape(NB, 128)
        sh = sh.reshape(NB, 128)
        for n in range(NB):
            p_ref[0, n] = jnp.broadcast_to(sc[n:n + 1], (8, 128))
            p_ref[1, n] = jnp.broadcast_to(sh[n:n + 1], (8, 128))
        for cp in wcopies(0):
            cp.wait()
        wtransform(0, v_ref.at[0], allr)

        def first_block(c, carry):
            for cp in xcopies(c):
                cp.wait()
            usv = us_ref.at[:, pl.ds(pl.multiple_of(c * RW, RW), RW), :]
            transform(c, usv, allp)
            Ms = {}
            for k in range(NB):
                for j in range(NJ):
                    m = mm(usv[j, :, k * 128:(k + 1) * 128], vsrc(j, 0)[k * 64:(k + 1) * 64, :])
                    Ms[j] = m if k == 0 else Ms[j] + m
            epi(c, 0, Ms)
            return carry

        lax.fori_loop(0, NSC, first_block, 0)

        for cp in wcopies(1):
            cp.wait()
        for gi, (gp, gr) in enumerate(W1G):
            if gp is None:
                wtransform(1, v_ref.at[1], split(allr, gi, len(W1G)))
        for j in range(3):
            m = mm(us_ref[j], vsrc(j, 1)[...])
            mr_ref[j] = m
            for gi, (gp, gr) in enumerate(W1G):
                if gp == j:
                    wtransform(1, v_ref.at[1], split(allr, gi, len(W1G)),
                               zero_from(m[gr:gr + 8]))

        def step(r, carry):
            for cp in wcopies(r):
                cp.wait()
            v2 = v_ref.at[pl.ds(r - 1, 2)]
            for gi, (gp, gr) in enumerate(SGATE):
                if gp is None:
                    wtransform(r, v2.at[1], split(allr, gi, len(SGATE)))
            Ms = {j: mr_ref[j] for j in range(3)}
            raws = {}
            for pos, j in enumerate(SORD):
                if j < 3:
                    m = raws[j] = mm(us_ref[j], vsrc(j, r)[...])
                else:
                    m = Ms[j] = mm(us_ref[j], vsrc(j, r - 1, v2.at[0])[...])
                for gi, (gp, gr) in enumerate(SGATE):
                    if gp == pos:
                        wtransform(r, v2.at[1], split(allr, gi, len(SGATE)),
                                   zero_from(m[gr:gr + 8]))
            for c in range(NSC):
                epi(c, r - 1, {j: Ms[j][c * TB:(c + 1) * TB] for j in range(NJ)})
            for j in range(3):
                mr_ref[j] = raws[j]
            return carry

        lax.fori_loop(2, NB, step, 0)

        for cp in xcopies(NSC):
            cp.wait()
        for gi, (gp, gr) in enumerate(FGATE):
            if gp is None:
                transform(NSC, ua_ref, split(allp, gi, len(FGATE)))
        for c in range(NSC):
            Ms = {j: mr_ref[j, c * TB:(c + 1) * TB] for j in range(3)}
            for pos, j in enumerate(FORD):
                Ms[j] = mm(us_ref[j, c * RW:(c + 1) * RW, :], vsrc(j, NB - 1)[...])
                for gi, (gp, gr) in enumerate(FGATE):
                    if gp == pos + len(FORD) * c:
                        transform(NSC, ua_ref, split(allp, gi, len(FGATE)),
                                  zero_from(Ms[j][gr:gr + 8]))
            epi(c, NB - 1, Ms)
        for k in range(NB):
            ocopy(0, NSC * TM, k).start()

        def group(gi, carry):
            a = NSC + UN * gi
            for cp in xcopies(a + 1):
                cp.wait()

            @pl.when(a + 2 < NC)
            def _():
                for cp in xcopies(a + 2):
                    cp.wait()

            for u in range(UN):
                i = a + u
                inext = jnp.minimum(i + 1, NC - 1)
                ucur, unext = (ua_ref, ub_ref) if u == 0 else (ub_ref, ua_ref)
                for n in range(NB):
                    Ms = {}
                    for pos, j in enumerate(JORD):
                        Ms[j] = mm(ucur[j], vsrc(j, n)[...])
                        for q, (gp, gr) in enumerate(TGATE):
                            if gp == pos:
                                transform(inext, unext, [(n, q)], zero_from(Ms[j][gr:gr + 8]))
                    epi(i, n, Ms)
                    ocopy(i * TM, TM, n).start()
            for d in range(UN):
                @pl.when(a + 1 + UN * XPRE + d < NC)
                def _():
                    issue_x(a + 1 + UN * XPRE + d, 0)
            return carry

        lax.fori_loop(0, NG, group, 0)
        pltpu.make_async_copy(o_hbm, o_hbm, so.at[0]).wait()

    anyspec = pl.BlockSpec(memory_space=pl.ANY)
    out = pl.pallas_call(
        kernel,
        grid=(1,),
        in_specs=[anyspec] * 6,
        out_specs=anyspec,
        out_shape=jax.ShapeDtypeStruct((B * S, C), x.dtype),
        scratch_shapes=[
            pltpu.VMEM((NB, B * S, 128), bf16),
            pltpu.VMEM((NB, B * S, 128), bf16),
            pltpu.VMEM((3, NB, C, 128), bf16),
            pltpu.VMEM((NB, 4, C // 2, 256), u32),
            pltpu.VMEM((NJ, RW, C), u32),
            pltpu.VMEM((NJ, RW, C), u32),
            pltpu.VMEM((NJ, NSC * RW, C), u32),
            pltpu.VMEM((3, NSC * TB, 128), f32),
            pltpu.VMEM((C,), bf16), pltpu.VMEM((C,), bf16),
            pltpu.VMEM((C,), bf16), pltpu.VMEM((C,), bf16),
            pltpu.VMEM((2, NB, 8, 128), f32),
            pltpu.VMEM((NPK, TB // 2, 256), u32),
            pltpu.SemaphoreType.DMA((NC,)),
            pltpu.SemaphoreType.DMA((1,)),
            pltpu.SemaphoreType.DMA((NB,)),
            pltpu.SemaphoreType.DMA((1,)),
        ],
        compiler_params=_compiler_params(),
    )(x.reshape(B * S, C), w, mean, var, g, b)
    return out.reshape(B, S, C)
```
